```python
import jax
import jax.numpy as jnp

def _softmax(x, axis=-1):
    return jax.nn.softmax(x, axis=axis)
def _gelu(x):
    return jax.nn.gelu(x, approximate=True)
def _silu(x):
    return jax.nn.silu(x)
def _sigmoid(x):
    return jax.nn.sigmoid(x)
def _layernorm(x, axis=-1, eps=1e-5):
    m = jnp.mean(x, axis=axis, keepdims=True)
    v = jnp.var(x, axis=axis, keepdims=True)
    return (x - m) / jnp.sqrt(v + eps)
def _scatter_add(tgt, idx, src, axis=0):
    return tgt.at[idx].add(src)
def _segment_sum(src, seg, n):
    return jax.ops.segment_sum(src, seg, n)
class _Rng:
    def __init__(self, key):
        self._k = key
    def _next(self):
        self._k, sub = jax.random.split(self._k)
        return sub
    def normal(self, shape):
        return jax.random.normal(self._next(), shape, dtype=jnp.bfloat16)
    def randint(self, lo, hi, shape):
        return jax.random.randint(self._next(), shape, lo, hi, dtype=jnp.int32)
    def uniform(self, shape, lo=0.0, hi=1.0):
        return jax.random.uniform(self._next(), shape, jnp.bfloat16, lo, hi)
    def permutation(self, n):
        return jax.random.permutation(self._next(), n)


kernel_name = 'interleave_layers__sliding_local_dilated__mixer_token_mlp__prompt'

def setup_inputs():
    _rng = _Rng(jax.random.key(int.from_bytes(__import__("os").urandom(4), "little")))
    _w = (lambda a: (lambda t: t.astype(jnp.bfloat16) if jnp.issubdtype(t.dtype, jnp.floating) else t)(jnp.asarray(a)))
    def _A_setup():
        B, S, D = 1, 2048, 1024
        return {
            "x": _w((lambda *s: _rng.normal(s) * 0.05)(B, S, D)),
            "wqkv": _w((lambda *s: _rng.normal(s) * 0.05)(D, 3 * D)),
            "wo": _w((lambda *s: _rng.normal(s) * 0.05)(D, D)),
        }
    _A_in = _A_setup()

    def _B_setup():
        B, S, D, F = 1, 2048, 1024, 3584
        return {
            "x": _w((lambda *s: _rng.normal(s) * 0.05)(B, S, D)),
            "w1": _w((lambda *s: _rng.normal(s) * 0.05)(S, F) * (S ** -0.5)),
            "b1": _w((lambda *s: _rng.normal(s) * 0.05)(F) * 0.02),
            "w2": _w((lambda *s: _rng.normal(s) * 0.05)(F, S) * (F ** -0.5)),
            "b2": _w((lambda *s: _rng.normal(s) * 0.05)(S) * 0.02),
        }
    _B_in = _B_setup()

    return {
        "A_x": _A_in["x"],
        "A_wqkv": _A_in["wqkv"],
        "A_wo": _A_in["wo"],
        "B_x": _B_in["x"],
        "B_w1": _B_in["w1"],
        "B_b1": _B_in["b1"],
        "B_w2": _B_in["w2"],
        "B_b2": _B_in["b2"],
    }

def reference(A_x, A_wqkv, A_wo, B_x, B_w1, B_b1, B_w2, B_b2):
    def _A_ref(x, wqkv, wo):
        B, S, D = x.shape
        H = 32; Dh = D // H
        W, dil = 8, 2
        qkv = (lambda x, *d: x.transpose(*d))((x @ wqkv).reshape(B, S, 3, H, Dh), 2, 0, 3, 1, 4)
        q, k, v = qkv[0], qkv[1], qkv[2]
        scale = Dh ** -0.5
        pos = jnp.arange(S)
        off = jnp.arange(W) * dil
        idx = pos[:, None] - off[None, :]
        mask = idx >= 0
        idx_c = jnp.where(mask, idx, 0).reshape(-1)
        kg = k[:, :, idx_c, :].reshape(B, H, S, W, Dh)
        vg = v[:, :, idx_c, :].reshape(B, H, S, W, Dh)
        logits = jnp.einsum("bhsd,bhswd->bhsw", q, kg) * scale
        logits = jnp.where(mask[None, None, :, :], logits, -1e9)
        attn = _softmax(logits, axis=-1)
        o = jnp.einsum("bhsw,bhswd->bhsd", attn, vg)
        return (lambda x, *d: x.transpose(*d))(o, 0, 2, 1, 3).reshape(B, S, D) @ wo

    def _B_ref(x, w1, b1, w2, b2):
        B, S, D = x.shape
        h = _layernorm(x, axis=-1)
        u = jnp.einsum("bsd,sf->bdf", h, w1) + b1
        u = _gelu(u)
        y = jnp.einsum("bdf,fs->bds", u, w2) + b2
        return (lambda x, *d: x.transpose(*d))(y, 0, 2, 1)

    x = A_x
    x = x + _A_ref(_layernorm(x, axis=-1), A_wqkv, A_wo)
    x = x + _B_ref(_layernorm(x, axis=-1), B_w1, B_b1, B_w2, B_b2)
    x = x + _A_ref(_layernorm(x, axis=-1), A_wqkv, A_wo)
    x = x + _B_ref(_layernorm(x, axis=-1), B_w1, B_b1, B_w2, B_b2)
    return x
```

```python
import functools
import jax
import jax.numpy as jnp
from jax import lax
import jax.experimental.pallas as pl
import jax.experimental.pallas.tpu as pltpu

S, D, F = 2048, 1024, 3584
T = 256
NC = S // T
FC = 512
NF = F // FC
W, DIL, DH = 8, 2, 32
HALO = 16
EPS = 1e-5
RG = 16
LOG2E = 1.4426950408889634
f32, bf16 = jnp.float32, jnp.bfloat16


def _dot(a, b):
    return lax.dot_general(a, b, (((1,), (0,)), ((), ())), preferred_element_type=f32)


def _dot_nt(a, b):
    return lax.dot_general(a, b, (((1,), (1,)), ((), ())), preferred_element_type=f32)


def _gelu(x):
    c = 0.7978845608028654
    inner = x * (c + (c * 0.044715) * (x * x))
    return (0.5 * x) * (1.0 + jnp.tanh(inner))


def _kernel(x_hbm, wqkv_hbm, wo_hbm, w1_hbm, b1_ref, w2_hbm, b2_ref, out_hbm,
            xio, x_s, wqkv_p, wo_raw, wo_p, w1_s, w2_s, hT_s, u_s, q_s, k_s, v_s, h_s, o_s, y_s,
            sem_x, sem_wqkv, sem_wo, sem_w1, sem_w2, sem_out):
    def rows(i):
        return pl.ds(pl.multiple_of(i * T, T), T)

    cp_x = pltpu.make_async_copy(x_hbm, xio, sem_x)
    cp_wqkv = [pltpu.make_async_copy(wqkv_hbm.at[:, pl.ds(t * D, D)], u_s.at[:, pl.ds(t * D, D)], sem_wqkv.at[t])
               for t in range(3)]
    cp_wo = pltpu.make_async_copy(wo_hbm, wo_raw, sem_wo)
    cp_w1 = [pltpu.make_async_copy(w1_hbm.at[:, pl.ds(j * FC, FC)], w1_s.at[j], sem_w1.at[j]) for j in range(NF)]
    cp_w2 = [pltpu.make_async_copy(w2_hbm.at[:, pl.ds(i * T, T)], w2_s.at[i], sem_w2.at[i]) for i in range(NC)]
    for c in cp_wqkv:
        c.start()
    cp_x.start()
    cp_wo.start()
    for c in cp_w1 + cp_w2:
        c.start()

    for t in range(3):
        cp_wqkv[t].wait()
        for cb in range(D // 128):
            blk = u_s[:, t * D + cb * 128: t * D + (cb + 1) * 128].astype(f32)
            bt = blk.T
            for j in range(8):
                k_s[j, cb * 128:(cb + 1) * 128, :] = bt[:, j * 128:(j + 1) * 128]
        for d in range(DH):
            for j in range(8):
                wqkv_p[t * D + d * 32: t * D + (d + 1) * 32, j * 128:(j + 1) * 128] = k_s[j, pl.ds(d, 32, stride=32), :].astype(bf16)
    cp_wo.wait()
    for j in range(8):
        v_s[j, 0:D, :] = wo_raw[:, j * 128:(j + 1) * 128].astype(f32)
    for d in range(DH):
        for j in range(8):
            wo_p[d * 32:(d + 1) * 32, j * 128:(j + 1) * 128] = v_s[j, pl.ds(d, 32, stride=32), :].astype(bf16)
    cp_x.wait()
    x_s[...] = xio[...].astype(f32)
    k_s[:, 0:HALO, :] = jnp.zeros((8, HALO, 128), f32)

    def stats(x):
        m = jnp.mean(x, axis=-1, keepdims=True)
        xc = x - m
        v = jnp.mean(xc * xc, axis=-1, keepdims=True)
        return xc, v

    def stage_p(i):
        for g in range(T // 32):
            r = pl.ds(pl.multiple_of(i * T + g * 32, 32), 32)
            xc, v = stats(x_s[r, :])
            h_s[g * 32:(g + 1) * 32, :] = (xc * lax.rsqrt(v + EPS)).astype(bf16)

    def stage_q(i):
        h = h_s[...]
        r = pl.ds(pl.multiple_of(i * T, T), T)
        rh = pl.ds(pl.multiple_of(i * T + HALO, HALO), T)
        q_s[r, :] = _dot_nt(h, wqkv_p[0:D, :]) * (DH ** -0.5 * LOG2E)
        k = _dot_nt(h, wqkv_p[D:2 * D, :])
        for j in range(8):
            k_s[j, rh, :] = k[:, j * 128:(j + 1) * 128]
        v = _dot_nt(h, wqkv_p[2 * D:3 * D, :])
        for j in range(8):
            v_s[j, rh, :] = v[:, j * 128:(j + 1) * 128]

    def stage_a(i, first):
        if first:
            v_s[:, 0:HALO, :] = jnp.broadcast_to(v_s[:, HALO:HALO + 1, :], (8, HALO, 128))
        for g in range(T // RG):
            base = i * T + g * RG
            q = [q_s[pl.ds(pl.multiple_of(base, RG), RG), j * 128:(j + 1) * 128] for j in range(8)]
            lg = []
            for w in range(W):
                rs = pl.ds(base + (HALO - DIL * w), RG)
                acc = None
                for j in range(8):
                    p = q[j] * k_s[j, rs, :]
                    acc = p if acc is None else acc + p
                acc = acc + pltpu.roll(acc, 64, 1)
                acc = acc + pltpu.roll(acc, 32, 1)
                if first and g * RG < DIL * w:
                    pos = lax.broadcasted_iota(jnp.int32, (RG, 128), 0) + g * RG
                    acc = jnp.where(pos >= DIL * w, acc, -1e9 * LOG2E)
                lg.append(acc)
            m = functools.reduce(jnp.maximum, lg)
            e = [jnp.exp2(l - m) for l in lg]
            inv = 1.0 / functools.reduce(jnp.add, e)
            p = [x * inv for x in e]
            for j in range(8):
                acc = None
                for w in range(W):
                    rs = pl.ds(base + (HALO - DIL * w), RG)
                    t = p[w] * v_s[j, rs, :]
                    acc = t if acc is None else acc + t
                o_s[pl.ds(pl.multiple_of(base, RG), RG), j * 128:(j + 1) * 128] = acc.astype(bf16)

    def stage_o(i):
        y = _dot(o_s[rows(i), :], wo_p[...])
        for g in range(T // 128):
            r = pl.ds(pl.multiple_of(i * T + g * 128, 128), 128)
            x = x_s[r, :] + y[g * 128:(g + 1) * 128, :]
            x_s[r, :] = x
            xc, v = stats(x)
            r1 = lax.rsqrt(v + EPS)
            r2 = lax.rsqrt(v * (r1 * r1) + EPS)
            h = (xc * (r1 * r2)).astype(bf16)
            hT_s[:, pl.ds(pl.multiple_of(i * T + g * 128, 128), 128)] = h.T

    def layer(l, carry):
        stage_p(0)
        stage_q(0)
        stage_p(1)
        stage_q(1)
        stage_a(0, True)

        def body(i, c):
            stage_o(i - 1)
            stage_p(i + 1)
            stage_q(i + 1)
            stage_a(i, False)
            return c
        lax.fori_loop(1, NC - 1, body, 0)
        stage_o(NC - 2)
        stage_a(NC - 1, False)
        stage_o(NC - 1)

        @pl.when(l == 0)
        def _():
            for c in cp_w1 + cp_w2:
                c.wait()

        def body_u(j, c):
            cols = pl.ds(pl.multiple_of(j * FC, FC), FC)
            b = b1_ref[:, cols].astype(f32)
            for m in range(D // 256):
                z = _dot(hT_s[m * 256:(m + 1) * 256, :], w1_s[j]) + b
                u_s[m * 256:(m + 1) * 256, cols] = _gelu(z).astype(bf16)
            return c
        lax.fori_loop(0, NF, body_u, 0)

        def mm_y(i):
            y_s[...] = _dot(u_s[...], w2_s[i]) + b2_ref[:, rows(i)].astype(f32)

        def add_y(i):
            x = x_s[rows(i), :] + y_s[...].T
            x_s[rows(i), :] = x
            xio[rows(i), :] = x.astype(bf16)

        def out_copy(i):
            return pltpu.make_async_copy(xio.at[rows(i), :], out_hbm.at[rows(i), :], sem_out.at[i])

        mm_y(0)

        def body_y(i, c):
            add_y(i - 1)
            mm_y(i)

            @pl.when(l == 1)
            def _():
                out_copy(i - 1).start()
            return c
        lax.fori_loop(1, NC, body_y, 0)
        add_y(NC - 1)

        @pl.when(l == 1)
        def _():
            out_copy(NC - 1).start()
            for i in range(NC):
                out_copy(i).wait()
        return carry

    lax.fori_loop(0, 2, layer, 0)


@jax.jit
def pallas_interleave_layers__sliding_local_dilated__mixer_token_mlp__prompt_kernel(
        A_x, A_wqkv, A_wo, B_x, B_w1, B_b1, B_w2, B_b2):
    del B_x
    any_spec = pl.BlockSpec(memory_space=pl.ANY)
    vm = pl.BlockSpec(memory_space=pltpu.VMEM)
    out = pl.pallas_call(
        _kernel,
        out_shape=jax.ShapeDtypeStruct((S, D), bf16),
        in_specs=[any_spec, any_spec, any_spec, any_spec, vm, any_spec, vm],
        out_specs=any_spec,
        scratch_shapes=[
            pltpu.VMEM((S, D), bf16),
            pltpu.VMEM((S, D), f32),
            pltpu.VMEM((3 * D, D), bf16),
            pltpu.VMEM((D, D), bf16),
            pltpu.VMEM((D, D), bf16),
            pltpu.VMEM((NF, S, FC), bf16),
            pltpu.VMEM((NC, F, T), bf16),
            pltpu.VMEM((D, S), bf16),
            pltpu.VMEM((D, F), bf16),
            pltpu.VMEM((S, D), f32),
            pltpu.VMEM((8, S + HALO, 128), f32),
            pltpu.VMEM((8, S + HALO, 128), f32),
            pltpu.VMEM((T, D), bf16),
            pltpu.VMEM((S, D), bf16),
            pltpu.VMEM((D, T), f32),
            pltpu.SemaphoreType.DMA(()),
            pltpu.SemaphoreType.DMA((3,)),
            pltpu.SemaphoreType.DMA(()),
            pltpu.SemaphoreType.DMA((NF,)),
            pltpu.SemaphoreType.DMA((NC,)),
            pltpu.SemaphoreType.DMA((NC,)),
        ],
        compiler_params=pltpu.CompilerParams(vmem_limit_bytes=120 * 1024 * 1024),
    )(A_x.reshape(S, D), A_wqkv, A_wo, B_w1, B_b1.reshape(1, F), B_w2, B_b2.reshape(1, S))
    return out.reshape(1, S, D)
```

```python
import functools
import jax
import jax.numpy as jnp
from jax import lax
import jax.experimental.pallas as pl
import jax.experimental.pallas.tpu as pltpu

S, D, F = 2048, 1024, 3584
T = 256
NC = S // T
FC = 512
NF = F // FC
W, DIL, DH = 8, 2, 32
HALO = 16
EPS = 1e-5
NP = 256
RG = 8
LOG2E = 1.4426950408889634
f32, bf16 = jnp.float32, jnp.bfloat16


def _dot(a, b):
    return lax.dot_general(a, b, (((1,), (0,)), ((), ())), preferred_element_type=f32)


def _dot_nt(a, b):
    return lax.dot_general(a, b, (((1,), (1,)), ((), ())), preferred_element_type=f32)


def _gelu(x):
    c = 0.7978845608028654
    inner = x * (c + (c * 0.044715) * (x * x))
    return (0.5 * x) * (1.0 + jnp.tanh(inner))


def _kernel(x_hbm, wqkv_hbm, wo_hbm, w1_hbm, b1_ref, w2_hbm, b2_ref, out_hbm,
            xio, x_s, wqkv_p, wo_raw, wo_p, w1_s, w2_s, hT_s, u_s, q_s, k_s, v_s, h_s, h2_s, n_s, o_s, y_s, z_s, tmp,
            sem_x, sem_wqkv, sem_wo, sem_w1, sem_w2, sem_out):
    def rows(i):
        return pl.ds(pl.multiple_of(i * T, T), T)

    def x_copy(lo, hi, k):
        return pltpu.make_async_copy(x_hbm.at[lo * T:hi * T, :], xio.at[lo * T:hi * T, :], sem_x.at[k])

    cp_x = [x_copy(0, 1, 0), x_copy(1, 2, 1), x_copy(2, NC, 2)]
    cp_wqkv = [pltpu.make_async_copy(wqkv_hbm.at[:, pl.ds(t * D, D)], u_s.at[:, pl.ds(t * D, D)], sem_wqkv.at[t])
               for t in range(3)]
    cp_wo = pltpu.make_async_copy(wo_hbm, wo_raw, sem_wo)
    cp_w1 = [pltpu.make_async_copy(w1_hbm.at[:, pl.ds(j * FC, FC)], w1_s.at[j], sem_w1.at[j]) for j in range(NF)]
    cp_w2 = [pltpu.make_async_copy(w2_hbm.at[:, pl.ds(i * T, T)], w2_s.at[i], sem_w2.at[i]) for i in range(NC)]

    def perm_qkv(t):
        def piece(j):
            bt = u_s[j * 128:(j + 1) * 128, t * D:(t + 1) * D].astype(f32).T
            for hh in range(32):
                tmp[j, hh * 33:hh * 33 + 32, :] = bt[hh * 32:(hh + 1) * 32, :]
            for d in range(DH):
                r0 = (d // 4) * 384 + t * 128 + (d % 4) * 32
                wqkv_p[r0:r0 + 32, j * 128:(j + 1) * 128] = tmp[j, pl.ds(d, 32, stride=33), :].astype(bf16)
        return [functools.partial(piece, j) for j in range(8)]

    def perm_o():
        def piece(j):
            c = slice(j * 128, (j + 1) * 128)
            for hh in range(32):
                tmp[j, hh * 33:hh * 33 + 32, :] = wo_raw[hh * 32:(hh + 1) * 32, c].astype(f32)
            for d in range(DH):
                wo_p[d * 32:(d + 1) * 32, c] = tmp[j, pl.ds(d, 32, stride=33), :].astype(bf16)
        return [functools.partial(piece, j) for j in range(8)]

    def widen(lo, hi):
        def piece(i):
            x_s[i * T:(i + 1) * T, :] = xio[i * T:(i + 1) * T, :].astype(f32)
        return [functools.partial(piece, i) for i in range(lo, hi)]

    def stats(x):
        m = jnp.mean(x, axis=-1, keepdims=True)
        xc = x - m
        v = jnp.mean(xc * xc, axis=-1, keepdims=True)
        return xc, v

    def stage_p(i, h_s=h_s):
        def piece(g):
            r = pl.ds(pl.multiple_of(i * T + g * 32, 32), 32)
            xc, v = stats(x_s[r, :])
            h_s[g * 32:(g + 1) * 32, :] = (xc * lax.rsqrt(v + EPS)).astype(bf16)
        return [functools.partial(piece, g) for g in range(T // 32)]

    def stage_q(i, h_s=h_s):
        r = pl.ds(pl.multiple_of(i * T, T), T)
        rh = pl.ds(pl.multiple_of(i * T + HALO, HALO), T)

        hh = []
        def piece(j):
            if not hh: hh.append(h_s[...])
            y = _dot_nt(hh[0], wqkv_p[j * 384:(j + 1) * 384, :])
            q_s[r, j * 128:(j + 1) * 128] = y[:, 0:128] * (DH ** -0.5 * LOG2E)
            k_s[j, rh, :] = y[:, 128:256]
            v_s[j, rh, :] = y[:, 256:384]
        return [functools.partial(piece, n) for n in range(8)]

    def stage_a(i, first):
        def piece(g):
            if first and g == 0:
                v_s[:, 0:HALO, :] = jnp.broadcast_to(v_s[:, HALO:HALO + 1, :], (8, HALO, 128))
            base = i * T + g * RG
            q = [q_s[pl.ds(pl.multiple_of(base, RG), RG), j * 128:(j + 1) * 128] for j in range(8)]
            lg = []
            for w in range(W):
                rs = pl.ds(base + (HALO - DIL * w), RG)
                acc = None
                for j in range(8):
                    p = q[j] * k_s[j, rs, :]
                    acc = p if acc is None else acc + p
                acc = acc + pltpu.roll(acc, 64, 1)
                acc = acc + pltpu.roll(acc, 32, 1)
                if first and g * RG < DIL * w:
                    pos = lax.broadcasted_iota(jnp.int32, (RG, 128), 0) + g * RG
                    acc = jnp.where(pos >= DIL * w, acc, -1e9 * LOG2E)
                lg.append(acc)
            m = functools.reduce(jnp.maximum, lg)
            e = [jnp.exp2(l - m) for l in lg]
            inv = 1.0 / functools.reduce(jnp.add, e)
            p = [x * inv for x in e]
            for j in range(8):
                acc = None
                for w in range(W):
                    rs = pl.ds(base + (HALO - DIL * w), RG)
                    t = p[w] * v_s[j, rs, :]
                    acc = t if acc is None else acc + t
                o_s[pl.ds(pl.multiple_of(base, RG), RG), j * 128:(j + 1) * 128] = acc
        return [functools.partial(piece, g) for g in range(T // RG)]

    def stage_o(i):
        def piece(n):
            c = slice(n * NP, (n + 1) * NP)
            x_s[rows(i), c] = x_s[rows(i), c] + _dot(o_s[rows(i), :].astype(bf16), wo_p[:, c])
        return [functools.partial(piece, n) for n in range(D // NP)]

    def stage_n(i):
        def piece(g):
            r = pl.ds(pl.multiple_of(i * T + g * 32, 32), 32)
            xc, v = stats(x_s[r, :])
            r1 = lax.rsqrt(v + EPS)
            r2 = lax.rsqrt(v * (r1 * r1) + EPS)
            n_s[g * 32:(g + 1) * 32, :] = (xc * (r1 * r2)).astype(bf16)
            if g % 4 == 3:
                g0 = (g // 4) * 128
                hT_s[:, pl.ds(pl.multiple_of(i * T + g0, 128), 128)] = n_s[g0:g0 + 128, :].T
        return [functools.partial(piece, g) for g in range(T // 32)]

    def run(main, **spread):
        slots = [[] for _ in main]
        for pcs, lo, hi in spread.values():
            for n, pc in enumerate(pcs):
                slots[lo + n * (hi - lo) // len(pcs)].append(pc)
        for m, side in zip(main, slots):
            m()
            for pc in side:
                pc()

    nq, no = 8, D // NP

    def stage_q0(t):
        hh = []

        def piece(j):
            if not hh:
                hh.append(h2_s[...])
            y = _dot_nt(hh[0], wqkv_p[j * 384 + t * 128:j * 384 + (t + 1) * 128, :])
            if t == 0:
                q_s[0:T, j * 128:(j + 1) * 128] = y * (DH ** -0.5 * LOG2E)
            else:
                (k_s if t == 1 else v_s)[j, HALO:HALO + T, :] = y
        return [functools.partial(piece, j) for j in range(8)]

    KP = (NC - 2) * T

    def part_u():
        def piece(m):
            r = slice(m * 256, (m + 1) * 256)
            z_s[r, :] = _dot(hT_s[r, 0:KP], w1_s[0, 0:KP, :])
        return [functools.partial(piece, m) for m in range(D // 256)]

    def mm_y(i, lo=0, n=T):
        def piece(m):
            r = slice(m * 256, (m + 1) * 256)
            b = b2_ref[:, pl.ds(pl.multiple_of(i * T + lo, 128), n)].astype(f32)
            y_s[r, lo:lo + n] = _dot(u_s[r, :], w2_s[i, :, lo:lo + n]) + b
        return [functools.partial(piece, m) for m in range(D // 256)]

    def add_y(i, lo=0, n=T):
        r = pl.ds(pl.multiple_of(i * T + lo, 128), n)
        x = x_s[r, :] + y_s[:, lo:lo + n].T
        x_s[r, :] = x
        xio[r, :] = x.astype(bf16)

    def out_copy(i, lo=0, n=T, k=None):
        r = pl.ds(pl.multiple_of(i * T + lo, 128), n)
        return pltpu.make_async_copy(xio.at[r, :], out_hbm.at[r, :], sem_out.at[i if k is None else k])

    with jax.named_scope("init"):
        cp_x[0].start()
        cp_wqkv[0].start()
        k_s[:, 0:HALO, :] = jnp.zeros((8, HALO, 128), f32)
        cp_x[0].wait()
        cp_wqkv[1].start()
        run(widen(0, 1) + stage_p(0, h2_s))
        cp_wqkv[0].wait()
        cp_wqkv[2].start()
        cp_x[1].start()
        run(perm_qkv(0))
        cp_wqkv[1].wait()
        cp_wo.start()
        run(stage_q0(0), w=(perm_qkv(1), 0, 8))
        cp_wqkv[2].wait()
        cp_x[1].wait()
        cp_x[2].start()
        run(stage_q0(1), w=(perm_qkv(2), 0, 8))
        run(stage_q0(2), p=(widen(1, 2) + stage_p(1), 0, 8))
        cp_wo.wait()
        cp_x[2].wait()
        for c in cp_w1 + cp_w2:
            c.start()
        run(stage_q(1), a=(stage_a(0, True), 0, nq), w=(perm_o(), 0, nq), x=(widen(2, NC), 0, nq))

    def layer(l, carry):
        def body(i, c):
            run(stage_o(i - 1) + stage_q(i + 1),
                p=(stage_p(i + 1), 0, no - 1),
                n=(stage_n(i - 1), no, no + nq),
                a=(stage_a(i, False), no - 1, no + nq))
            return c
        with jax.named_scope("Aloop"):
            lax.fori_loop(1, NC - 1, body, 0)

        @pl.when(l == 0)
        def _():
            for c in cp_w1 + cp_w2:
                c.wait()

        with jax.named_scope("Aepi"):
            pu = part_u()
            run(stage_o(NC - 2) + pu[:2], a=(stage_a(NC - 1, False), 0, no + 2), n=(stage_n(NC - 2), no, no + 2))
            run(stage_o(NC - 1) + pu[2:], n=(stage_n(NC - 1), no, no + 2))
            for m in range(D // 256):
                r = slice(m * 256, (m + 1) * 256)
                z = z_s[r, :] + _dot(hT_s[r, KP:S], w1_s[0, KP:S, :]) + b1_ref[:, 0:FC].astype(f32)
                u_s[r, 0:FC] = _gelu(z).astype(bf16)

        def body_u(j, c):
            cols = pl.ds(pl.multiple_of(j * FC, FC), FC)
            b = b1_ref[:, cols].astype(f32)
            for m in range(D // 256):
                z = _dot(hT_s[m * 256:(m + 1) * 256, :], w1_s[j]) + b
                u_s[m * 256:(m + 1) * 256, cols] = _gelu(z).astype(bf16)
            return c
        with jax.named_scope("Uloop"):
            lax.fori_loop(1, NF, body_u, 0)

        def mm_full(i):
            y_s[...] = _dot(u_s[...], w2_s[i]) + b2_ref[:, rows(i)].astype(f32)

        with jax.named_scope("Ypro"):
            mm_full(0)

        def body_y(i, c):
            add_y(i - 1)
            mm_full(i)

            @pl.when(l == 1)
            def _():
                out_copy(i - 1).start()
            return c
        with jax.named_scope("Yloop"):
            lax.fori_loop(1, NC - 1, body_y, 0)

        with jax.named_scope("Mid"):
            @pl.when(l == 0)
            def _():
                add_y(NC - 2)
                run(mm_y(NC - 1), p=(stage_p(0, h2_s), 0, 2), p1=(stage_p(1), 2, 4))
                add_y(NC - 1)
                run(stage_q(0, h2_s))
                run(stage_q(1), a=(stage_a(0, True), 0, nq))

        with jax.named_scope("Tail"):
            @pl.when(l == 1)
            def _():
                add_y(NC - 2)
                run(mm_y(NC - 1, 0, 128))
                out_copy(NC - 2).start()
                add_y(NC - 1, 0, 128)
                run(mm_y(NC - 1, 128, 128))
                out_copy(NC - 1, 0, 128).start()
                add_y(NC - 1, 128, 128)
                out_copy(NC - 1, 128, 128, NC).start()
                for i in range(NC - 1):
                    out_copy(i).wait()
                out_copy(NC - 1, 0, 128).wait()
                out_copy(NC - 1, 128, 128, NC).wait()
        return carry

    layer(0, 0)
    layer(1, 0)


@jax.jit
def pallas_interleave_layers__sliding_local_dilated__mixer_token_mlp__prompt_kernel(
        A_x, A_wqkv, A_wo, B_x, B_w1, B_b1, B_w2, B_b2):
    del B_x
    any_spec = pl.BlockSpec(memory_space=pl.ANY)
    vm = pl.BlockSpec(memory_space=pltpu.VMEM)
    out = pl.pallas_call(
        _kernel,
        out_shape=jax.ShapeDtypeStruct((S, D), bf16),
        in_specs=[any_spec, any_spec, any_spec, any_spec, vm, any_spec, vm],
        out_specs=any_spec,
        scratch_shapes=[
            pltpu.VMEM((S, D), bf16),
            pltpu.VMEM((S, D), f32),
            pltpu.VMEM((3 * D, D), bf16),
            pltpu.VMEM((D, D), bf16),
            pltpu.VMEM((D, D), bf16),
            pltpu.VMEM((NF, S, FC), bf16),
            pltpu.VMEM((NC, F, T), bf16),
            pltpu.VMEM((D, S), bf16),
            pltpu.VMEM((D, F), bf16),
            pltpu.VMEM((S, D), f32),
            pltpu.VMEM((8, S + HALO, 128), f32),
            pltpu.VMEM((8, S + HALO, 128), f32),
            pltpu.VMEM((T, D), bf16),
            pltpu.VMEM((T, D), bf16),
            pltpu.VMEM((T, D), bf16),
            pltpu.VMEM((S, D), f32),
            pltpu.VMEM((D, T), f32),
            pltpu.VMEM((D, FC), f32),
            pltpu.VMEM((8, 32 * 33, 128), f32),
            pltpu.SemaphoreType.DMA((3,)),
            pltpu.SemaphoreType.DMA((3,)),
            pltpu.SemaphoreType.DMA(()),
            pltpu.SemaphoreType.DMA((NF,)),
            pltpu.SemaphoreType.DMA((NC,)),
            pltpu.SemaphoreType.DMA((NC + 1,)),
        ],
        compiler_params=pltpu.CompilerParams(vmem_limit_bytes=120 * 1024 * 1024),
    )(A_x.reshape(S, D), A_wqkv, A_wo, B_w1, B_b1.reshape(1, F), B_w2, B_b2.reshape(1, S))
    return out.reshape(1, S, D)
```
